```python
import os as _os
_os.environ.setdefault("JAX_PLATFORMS", "cpu")
import jax
import jax.numpy as jnp

def _softmax(x, axis=-1):
    return jax.nn.softmax(x, axis=axis)
def _gelu(x):
    return jax.nn.gelu(x, approximate=True)
def _silu(x):
    return jax.nn.silu(x)
def _sigmoid(x):
    return jax.nn.sigmoid(x)
def _layernorm(x, axis=-1, eps=1e-5):
    m = jnp.mean(x, axis=axis, keepdims=True)
    v = jnp.var(x, axis=axis, keepdims=True)
    return (x - m) / jnp.sqrt(v + eps)
def _scatter_add(tgt, idx, src, axis=0):
    return tgt.at[idx].add(src)
def _segment_sum(src, seg, n):
    return jax.ops.segment_sum(src, seg, n)
class _Rng:
    def __init__(self, key):
        self._k = key
    def _next(self):
        self._k, sub = jax.random.split(self._k)
        return sub
    def normal(self, shape):
        return jax.random.normal(self._next(), shape, dtype=jnp.bfloat16)
    def randint(self, lo, hi, shape):
        return jax.random.randint(self._next(), shape, lo, hi, dtype=jnp.int32)
    def uniform(self, shape, lo=0.0, hi=1.0):
        return jax.random.uniform(self._next(), shape, jnp.bfloat16, lo, hi)
    def permutation(self, n):
        return jax.random.permutation(self._next(), n)


kernel_name = 'gated_mix__sliding_block__dense_activation_silu__prompt'

def setup_inputs():
    _rng = _Rng(jax.random.key(int.from_bytes(__import__("os").urandom(4), "little")))
    _w = (lambda a: (lambda t: t.astype(jnp.bfloat16) if jnp.issubdtype(t.dtype, jnp.floating) else t)(jnp.asarray(a)))
    def _A_setup():
        B, S, D = 1, 2048, 640
        return {
            "x": _w((lambda *s: _rng.normal(s) * 0.05)(B, S, D)),
            "wqkv": _w((lambda *s: _rng.normal(s) * 0.4)(D, 3 * D)),
            "wo": _w((lambda *s: _rng.normal(s) * 0.05)(D, D)),
        }
    _A_in = _A_setup()

    def _B_setup():
        B, S, D, F = 1, 2048, 640, 1536
        return {
            "x": _w((lambda *s: _rng.normal(s) * 0.05)(B, S, D)),
            "w1": _w((lambda *s: _rng.normal(s) * 1.6)(D, F) * (D ** -0.5)),
            "w2": _w((lambda *s: _rng.normal(s) * 1.6)(F, D) * (F ** -0.5)),
        }
    _B_in = _B_setup()

    return {
        "A_x": _A_in["x"],
        "A_wqkv": _A_in["wqkv"],
        "A_wo": _A_in["wo"],
        "B_x": _B_in["x"],
        "B_w1": _B_in["w1"],
        "B_w2": _B_in["w2"],
        "gate_w": _w((lambda *s: _rng.normal(s) * 0.05)(640) * 16.0),
    }

def reference(A_x, A_wqkv, A_wo, B_x, B_w1, B_w2, gate_w):
    def _A_ref(x, wqkv, wo):
        B, S, D = x.shape
        H = 32; Dh = D // H; W = 256
        qkv = (lambda x, *d: x.transpose(*d))((x @ wqkv).reshape(B, S, 3, H, Dh), 2, 0, 3, 1, 4)
        q, k, v = qkv[0], qkv[1], qkv[2]
        scores = jnp.einsum("bhqd,bhkd->bhqk", q, k) * (Dh ** -0.5)
        idx = jnp.arange(S)
        mask = (idx[:, None] - idx[None, :] >= 0) & (idx[:, None] - idx[None, :] < W)
        scores = jnp.where(mask[None, None], scores, -1e9)
        p = _softmax(scores, axis=-1)
        o = jnp.einsum("bhqk,bhkd->bhqd", p, v)
        return (lambda x, *d: x.transpose(*d))(o, 0, 2, 1, 3).reshape(B, S, D) @ wo

    def _B_ref(x, w1, w2):
        h = jnp.einsum("bsd,df->bsf", x, w1)
        h = _silu(h)
        out = jnp.einsum("bsf,fd->bsd", h, w2)
        return out

    x = A_x
    g = _sigmoid((x * gate_w).sum(-1, keepdims=True))
    a = _A_ref(x, A_wqkv, A_wo)
    b = _B_ref(x, B_w1, B_w2)
    return g * a + (1 - g) * b
```

```python
import jax
import jax.numpy as jnp
import numpy as np
from jax import lax
from jax.experimental import pallas as pl
from jax.experimental.pallas import tpu as pltpu

S, D, H, DH, WIN, F = 2048, 640, 32, 20, 256, 1536
NSUB = 2
TQ = 128 * NSUB
NSTEP = S // TQ
LOG2E = 1.4426950408889634
NT = (((1,), (1,)), ((), ()))
NEG = -1e30
NG = 8
PMODE = "std"
FLAGS = {k: True for k in "".split(",") if k}
f32, bf16, i32 = jnp.float32, jnp.bfloat16, jnp.int32

OFFS = [0, 80 - 64, 160 - 128, 240 - 192, 320 - 320, 400 - 384, 480 - 448, 560 - 512]

def _regroup(a):
    lane = lax.broadcasted_iota(i32, (a.shape[0], 128), 1)
    t = [a[:, 128 * n:128 * (n + 1)] for n in range(5)]
    r = [pltpu.roll(x, 64, 1) for x in t]
    lo = lane < 64
    sh = [jnp.where(lo, r[n], r[n + 1]) for n in range(4)]
    return [t[0], sh[0], t[1], sh[1], sh[2], t[3], sh[3], t[4]]

def _pack(a, b):
    return pltpu.pack_elementwise([a, b], packed_dtype=bf16)

def _mm(a, b):
    return jnp.dot(a, b, preferred_element_type=f32)

SX, SWK, SWQ, SWV, SWO, SW2, SW1, SOUT = 0, NSTEP, NSTEP + 1, NSTEP + 2, NSTEP + 3, NSTEP + 4, NSTEP + 5, NSTEP + 8
NSEM = SOUT + NSTEP
W1C = 512

def kernel(x_hbm, wqkv_hbm, wo_hbm, w1_hbm, w2_hbm, gw_ref, o_hbm,
           x_v, wq_v, wk_v, wv_v, wo_v, w1_v, w2_v, o_v, sems,
           k_scr, vt_scr, wvt_scr, q_scr, s_scr, h_scr, b_scr, ot_scr, m_scr):

    def x_copy(i):
        r = pl.ds(pl.multiple_of(i * TQ, TQ), TQ)
        return pltpu.make_async_copy(x_hbm.at[r, :], x_v.at[r, :], sems.at[SX + i])
    def o_copy(i):
        r = pl.ds(pl.multiple_of(i * TQ, TQ), TQ)
        return pltpu.make_async_copy(o_v.at[r, :], o_hbm.at[r, :], sems.at[SOUT + i])
    cp_wk = pltpu.make_async_copy(wqkv_hbm.at[:, D:2 * D], wk_v, sems.at[SWK])
    cp_wq = pltpu.make_async_copy(wqkv_hbm.at[:, 0:D], wq_v, sems.at[SWQ])
    cp_wv = pltpu.make_async_copy(wqkv_hbm.at[:, 2 * D:3 * D], wv_v, sems.at[SWV])
    cp_wo = pltpu.make_async_copy(wo_hbm, wo_v, sems.at[SWO])
    cp_w2 = pltpu.make_async_copy(w2_hbm, w2_v, sems.at[SW2])
    cp_w1 = [pltpu.make_async_copy(w1_hbm.at[:, W1C * c:W1C * (c + 1)], w1_v.at[:, W1C * c:W1C * (c + 1)], sems.at[SW1 + c]) for c in range(F // W1C)]

    x_copy(0).start(); cp_wk.start(); cp_wq.start(); cp_wv.start()
    for c in cp_w1: c.start()
    cp_wo.start(); cp_w2.start()
    for i in range(1, NSTEP):
        x_copy(i).start()

    if PMODE == "pack":
        r = lax.broadcasted_iota(i32, (64, 128), 0)
        c = lax.broadcasted_iota(i32, (64, 128), 1)
        rlo = (r >> 3) * 16 + (r & 7)
        m_scr[...] = jnp.where(rlo <= c, 0xFFFF, 0) | jnp.where(rlo + 8 <= c, -65536, 0)

    def step(i, first):
        t0 = i * TQ if first else pl.multiple_of(i * TQ, TQ)
        lane = lax.broadcasted_iota(i32, (128, 128), 1)
        sub16 = lax.broadcasted_iota(i32, (16, 128), 0)
        lane16 = lax.broadcasted_iota(i32, (16, 128), 1)
        sub8 = lax.broadcasted_iota(i32, (8, 128), 0)
        st8 = {}
        xs = lambda: x_v[pl.ds(t0, TQ), :]

        def kproj():
            if first: cp_wk.wait()
            kg = _regroup(_mm(xs(), wk_v[...]))
            for j in range(NG):
                k_scr[pl.ds(t0, TQ), 128 * j:128 * (j + 1)] = kg[j].astype(bf16)

        def qproj():
            if first: cp_wq.wait()
            qg = _regroup(_mm(xs(), wq_v[...]) * (DH ** -0.5 * LOG2E))
            for j in range(NG):
                q_scr[j] = qg[j]

        def vproj():
            if first:
                cp_wv.wait()
                wvt_scr[...] = wv_v[...].astype(f32).T.astype(bf16)
            if PMODE == "pack":
                xf = xs().astype(f32)
                xp = pltpu.bitcast(jnp.concatenate([_pack(xf[16 * c:16 * c + 8], xf[16 * c + 8:16 * c + 16]) for c in range(TQ // 16)], axis=0), bf16)
            else:
                xp = xs()
            vt_scr[:, pl.ds(t0, TQ)] = lax.dot_general(wvt_scr[...], xp, NT, preferred_element_type=f32).astype(bf16)

        def ntile(sb):
            return min(3, sb + 1) if first else 3

        def qk(u):
            sb, j = u
            nt = ntile(sb)
            tq = t0 + 128 * sb
            kt = lambda r0, n: k_scr[pl.ds(tq + r0, n), 128 * j:128 * (j + 1)]
            if nt == 3:
                parts = []
                for c in range(8):
                    parts += [kt(16 * c - 256, 16), kt(16 * c, 16)]
                parts.append(kt(-128, 128))
            elif nt == 2:
                parts = [kt(0, 128), kt(-128, 128)]
            else:
                parts = [kt(0, 128)]
            kw = jnp.concatenate(parts, axis=0)
            qv = q_scr[j, 128 * sb:128 * (sb + 1), :]
            q4 = jnp.concatenate([jnp.where((lane >= OFFS[j] + DH * n) & (lane < OFFS[j] + DH * (n + 1)), qv, 0.0).astype(bf16) for n in range(4)], axis=0)
            st = lax.dot_general(kw, q4, NT, preferred_element_type=f32)
            mx = None
            b = (sb * NG + j) % 2
            for c in range(8):
                tri4 = jnp.concatenate([(sub16 + 16 * c) <= lane16] * 4, axis=1)
                if nt == 3:
                    s1 = jnp.where(tri4, st[32 * c + 16:32 * c + 32], st[32 * c:32 * c + 16])
                else:
                    s1 = jnp.where(tri4, st[16 * c:16 * c + 16], NEG)
                s_scr[b, 16 * c:16 * c + 16, :] = s1
                s1m = jnp.maximum(s1[0:8], s1[8:16])
                mx = s1m if mx is None else jnp.maximum(mx, s1m)
            if nt >= 2:
                base = 256 if nt == 3 else 128
                for c in range(8):
                    s2 = st[base + 16 * c:base + 16 * c + 16]
                    s_scr[b, 128 + 16 * c:128 + 16 * c + 16, :] = s2
                    mx = jnp.maximum(mx, jnp.maximum(s2[0:8], s2[8:16]))
            st8[("m", u)] = jnp.max(mx, axis=0, keepdims=True)

        def softmax(u):
            sb, j = u
            nt = ntile(sb)
            b = (sb * NG + j) % 2
            m = st8[("m", u)]
            acc = None
            far, mid, dia = [], [], []
            for c in range(8):
                p = jnp.exp2(s_scr[b, 16 * c:16 * c + 16, :] - m)
                if PMODE == "pack":
                    w = _pack(p[0:8], p[8:16])
                    if nt == 3:
                        wd = w & jnp.concatenate([m_scr[8 * c:8 * c + 8, :]] * 4, axis=1)
                        dia.append(wd)
                        far.append(w ^ wd)
                    else:
                        dia.append(w)
                else:
                    if nt == 3:
                        tri4 = jnp.concatenate([(sub16 + 16 * c) <= lane16] * 4, axis=1)
                        dia.append(jnp.where(tri4, p, 0.0))
                        far.append(jnp.where(tri4, 0.0, p))
                    else:
                        dia.append(p)
                ps = p[0:8] + p[8:16]
                acc = ps if acc is None else acc + ps
            if nt >= 2:
                for c in range(8):
                    p = jnp.exp2(s_scr[b, 128 + 16 * c:128 + 16 * c + 16, :] - m)
                    mid.append(_pack(p[0:8], p[8:16]) if PMODE == "pack" else p)
                    acc = acc + (p[0:8] + p[8:16])
            st8[("p", u)] = jnp.concatenate(far + mid + dia, axis=0)
            st8[("il", u)] = pl.reciprocal(jnp.sum(acc, axis=0, keepdims=True), approx=True)

        def pv(u):
            sb, j = u
            nt = ntile(sb)
            tq = t0 + 128 * sb
            il = st8[("il", u)]
            pw = st8[("p", u)]
            on = []
            for n in range(4):
                rb = ((4 * j + n) * DH // 16) * 16
                vw = vt_scr[rb:rb + 32, pl.ds(tq - 128 * (nt - 1), 128 * nt)]
                if PMODE == "pack":
                    ph = pltpu.bitcast(pw[:, 128 * n:128 * (n + 1)], bf16)
                else:
                    ph = pw[:, 128 * n:128 * (n + 1)].astype(bf16)
                on.append((rb, _mm(vw, ph) * il[:, 128 * n:128 * (n + 1)]))
            rows = []
            for r in range(10):
                r0 = 80 * j + 8 * r
                ha, hb = (8 * r) // DH, (8 * r + 7) // DH
                rba, oa = on[ha]
                va = oa[r0 - rba:r0 - rba + 8]
                if ha != hb:
                    rbb, ob = on[hb]
                    va = jnp.where(sub8 < (hb * DH - 8 * r), va, ob[r0 - rbb:r0 - rbb + 8])
                rows.append(va)
            ot_scr[80 * j:80 * j + 80, 128 * sb:128 * (sb + 1)] = jnp.concatenate(rows, axis=0)

        def gate():
            st8["g"] = jax.nn.sigmoid(jnp.sum(xs().astype(f32) * gw_ref[...].astype(f32), axis=-1, keepdims=True))

        def up(c):
            if first and (128 * c) % W1C == 0: cp_w1[128 * c // W1C].wait()
            hh2 = 0.5 * _mm(xs(), w1_v[:, 128 * c:128 * (c + 1)])
            h_scr[:, 128 * c:128 * (c + 1)] = (hh2 * jnp.tanh(hh2) + hh2).astype(bf16)

        def down(n):
            if first and n == 0: cp_w2.wait()
            b_scr[:, 128 * n:128 * (n + 1)] = (1.0 - st8["g"]) * _mm(h_scr[...], w2_v[:, 128 * n:128 * (n + 1)])

        def outproj(sb):
            if first and sb == 0: cp_wo.wait()
            r = slice(128 * sb, 128 * (sb + 1))
            o = ot_scr[:, r].T.astype(bf16)
            a = _mm(o, wo_v[...])
            o_v[pl.ds(t0 + 128 * sb, 128), :] = (st8["g"][r] * a + b_scr[r, :]).astype(bf16)

        units = [(sb, j) for sb in range(NSUB) for j in range(NG)]
        nu = len(units)
        prog = [kproj, qproj, vproj, gate, (qk, units[0])]
        fill = {k: [] for k in range(nu)}
        for c in range(12):
            fill[(c * (nu // 2)) // 12].append((up, c))
        dpos = [nu // 2 + (n * (nu // 2)) // 5 for n in range(5)]
        for n in range(5):
            fill[min(dpos[n] + (nu // 2) // 5, nu - 1)].append((down, n))
        for k in range(nu):
            if k + 1 < nu:
                prog.append((qk, units[k + 1]))
            prog.append((softmax, units[k]))
            prog += fill[k]
            prog.append((pv, units[k]))
        prog += [(outproj, sb) for sb in range(NSUB)]
        for p in prog:
            if isinstance(p, tuple):
                p[0](p[1])
            else:
                p()
        o_copy(i).start()

    x_copy(0).wait()
    step(0, True)
    def body(i, _):
        x_copy(i).wait()
        step(i, False)
        return _
    lax.fori_loop(1, NSTEP, body, 0)
    for i in range(NSTEP):
        o_copy(i).wait()


@jax.jit
def pallas_gated_mix__sliding_block__dense_activation_silu__prompt_kernel(A_x, A_wqkv, A_wo, B_x, B_w1, B_w2, gate_w):
    x = A_x.reshape(S, D)
    gw = gate_w.reshape(1, D)
    anyspec = pl.BlockSpec(memory_space=pl.ANY)
    out = pl.pallas_call(
        kernel,
        in_specs=[anyspec, anyspec, anyspec, anyspec, anyspec, pl.BlockSpec(memory_space=pltpu.VMEM)],
        out_specs=anyspec,
        out_shape=jax.ShapeDtypeStruct((S, D), bf16),
        scratch_shapes=[
            pltpu.VMEM((S, D), bf16),
            pltpu.VMEM((D, D), bf16),
            pltpu.VMEM((D, D), bf16),
            pltpu.VMEM((D, D), bf16),
            pltpu.VMEM((D, D), bf16),
            pltpu.VMEM((D, F), bf16),
            pltpu.VMEM((F, D), bf16),
            pltpu.VMEM((S, D), bf16),
            pltpu.SemaphoreType.DMA((NSEM,)),
            pltpu.VMEM((S, NG * 128), bf16),
            pltpu.VMEM((D, S), bf16),
            pltpu.VMEM((D, D), bf16),
            pltpu.VMEM((NG, TQ, 128), f32),
            pltpu.VMEM((2, 256, 512), f32),
            pltpu.VMEM((TQ, F), bf16),
            pltpu.VMEM((TQ, D), f32),
            pltpu.VMEM((D, TQ), f32),
            pltpu.VMEM((64, 128), i32),
        ],
        compiler_params=pltpu.CompilerParams(vmem_limit_bytes=100 * 1024 * 1024, flags=FLAGS or None),
    )(x, A_wqkv, A_wo, B_w1, B_w2, gw)
    return out.reshape(1, S, D)
```

```python
import jax
import jax.numpy as jnp
import numpy as np
from jax import lax
from jax.experimental import pallas as pl
from jax.experimental.pallas import tpu as pltpu

S, D, H, DH, WIN, F = 2048, 640, 32, 20, 256, 1536
NSUB = 2
TQ = 128 * NSUB
NSTEP = S // TQ
LOG2E = 1.4426950408889634
NT = (((1,), (1,)), ((), ()))
NEG = -1e30
NG = 8
PMODE = "std"
VMODE = "w"
FLAGS = {k: True for k in "".split(",") if k}
f32, bf16, i32 = jnp.float32, jnp.bfloat16, jnp.int32

OFFS = [0, 80 - 64, 160 - 128, 240 - 192, 320 - 320, 400 - 384, 480 - 448, 560 - 512]

def _regroup(a):
    lane = lax.broadcasted_iota(i32, (a.shape[0], 128), 1)
    t = [a[:, 128 * n:128 * (n + 1)] for n in range(5)]
    r = [pltpu.roll(x, 64, 1) for x in t]
    lo = lane < 64
    sh = [jnp.where(lo, r[n], r[n + 1]) for n in range(4)]
    return [t[0], sh[0], t[1], sh[1], sh[2], t[3], sh[3], t[4]]

def _roll(a, sh):
    sh %= 128
    return a if sh == 0 else pltpu.roll(a, sh, 1)

def _pack(a, b):
    return pltpu.pack_elementwise([a, b], packed_dtype=bf16)

def _mm(a, b):
    return jnp.dot(a, b, preferred_element_type=f32)

SX, SWK, SWQ, SWV, SWO, SW2, SW1, SOUT = 0, NSTEP, NSTEP + 1, NSTEP + 2, NSTEP + 3, NSTEP + 4, NSTEP + 5, NSTEP + 8
GW2D = "0" == "1"
ONES = "1" == "1"
LOOK = 1
NSEM = SOUT + S // 128
W1C = 512

def kernel(x_hbm, wqkv_hbm, wo_hbm, w1_hbm, w2_hbm, gw_ref, o_hbm,
           x_v, wq_v, wk_v, wv_v, wo_v, w1_v, w2_v, o_v, sems,
           k_scr, vt_scr, kraw_scr, q_scr, s_scr, h_scr, b_scr, ot_scr, m_scr):

    def x_copy(i):
        r = pl.ds(pl.multiple_of(i * TQ, TQ), TQ)
        return pltpu.make_async_copy(x_hbm.at[r, :], x_v.at[r, :], sems.at[SX + i])
    def o_copy(i):
        r = pl.ds(pl.multiple_of(i * 128, 128), 128)
        return pltpu.make_async_copy(o_v.at[r, :], o_hbm.at[r, :], sems.at[SOUT + i])
    cp_wk = pltpu.make_async_copy(wqkv_hbm.at[:, D:2 * D], wk_v, sems.at[SWK])
    cp_wq = pltpu.make_async_copy(wqkv_hbm.at[:, 0:D], wq_v, sems.at[SWQ])
    cp_wv = pltpu.make_async_copy(wqkv_hbm.at[:, 2 * D:3 * D], wv_v, sems.at[SWV])
    cp_wo = pltpu.make_async_copy(wo_hbm, wo_v, sems.at[SWO])
    cp_w2 = pltpu.make_async_copy(w2_hbm, w2_v, sems.at[SW2])
    cp_w1 = [pltpu.make_async_copy(w1_hbm.at[:, W1C * c:W1C * (c + 1)], w1_v.at[:, W1C * c:W1C * (c + 1)], sems.at[SW1 + c]) for c in range(F // W1C)]

    x_copy(0).start(); cp_wk.start(); cp_wq.start(); cp_wv.start()
    for c in cp_w1: c.start()
    cp_w2.start(); cp_wo.start()
    for i in range(1, NSTEP):
        x_copy(i).start()

    if PMODE == "pack":
        r = lax.broadcasted_iota(i32, (64, 128), 0)
        c = lax.broadcasted_iota(i32, (64, 128), 1)
        rlo = (r >> 3) * 16 + (r & 7)
        m_scr[...] = jnp.where(rlo <= c, 0xFFFF, 0) | jnp.where(rlo + 8 <= c, -65536, 0)

    def step(i, first):
        t0 = i * TQ if first else pl.multiple_of(i * TQ, TQ)
        lane = lax.broadcasted_iota(i32, (128, 128), 1)
        sub16 = lax.broadcasted_iota(i32, (16, 128), 0)
        lane16 = lax.broadcasted_iota(i32, (16, 128), 1)
        sub8 = lax.broadcasted_iota(i32, (8, 128), 0)
        lane8 = lax.broadcasted_iota(i32, (8, 128), 1)
        st8 = {}
        xs = lambda: x_v[pl.ds(t0, TQ), :]

        def kproj():
            kg = _regroup(_mm(xs(), wk_v[...]))
            for j in range(NG):
                kraw_scr[j] = pltpu.bitcast(kg[j].astype(bf16), i32)

        def k4(j):
            lanew = lax.broadcasted_iota(i32, (TQ // 2, 128), 1)
            kw_ = kraw_scr[j]
            for n in range(4):
                a = jnp.where(((lanew - (OFFS[j] + DH * n)) & 127) < DH, kw_, 0)
                a = a | _roll(a, DH)
                a = a | _roll(a, 2 * DH)
                for sb in range(NSUB):
                    k_scr[i * NSUB + sb, 4 * j + n] = a[64 * sb:64 * (sb + 1)]

        def qproj():
            qg = _regroup(_mm(xs(), wq_v[...]) * (DH ** -0.5 * LOG2E))
            for j in range(NG):
                q_scr[j] = pltpu.bitcast(qg[j].astype(bf16), i32)

        def vproj():
            if PMODE == "pack":
                xf = xs().astype(f32)
                xp = pltpu.bitcast(jnp.concatenate([_pack(xf[16 * c:16 * c + 8], xf[16 * c + 8:16 * c + 16]) for c in range(TQ // 16)], axis=0), bf16)
            else:
                xp = xs()
            vt = _mm(xp, wv_v[...]).T
            if ONES:
                row = lax.broadcasted_iota(i32, (32, TQ), 0)
                for h in range(H):
                    rb = (h * DH // 16) * 16
                    o = h * DH - rb
                    vt_scr[h, :, pl.ds(t0, TQ)] = jnp.where((row >= o) & (row < o + DH), vt[rb:rb + 32], 1.0).astype(bf16)
            else:
                vt_scr[:, pl.ds(t0, TQ)] = vt.astype(bf16)

        def ntile(sb):
            return min(3, sb + 1) if first else 3

        def qk(u):
            sb, j = u
            nt = ntile(sb)
            blk = i * NSUB + sb
            b = (sb * NG + j) % (LOOK + 1)
            lane16w = lax.broadcasted_iota(i32, (16, 128), 1)
            qv = q_scr[j, 64 * sb:64 * (sb + 1), :]
            ms = []
            for n in range(4):
                h = 4 * j + n
                rel = (lane16w - (OFFS[j] + DH * n)) & 127
                qw = jnp.concatenate([jnp.where((rel >= DH * v) & (rel < DH * (v + 1)), _roll(qv[16 * v:16 * v + 16], DH * v), 0) for v in range(4)], axis=0)
                qw = pltpu.bitcast(qw, bf16)
                kd = k_scr[blk, h]
                if nt == 3:
                    kf = k_scr[blk - 2, h]
                    ex = kf[0:16]
                    for v in range(1, 4):
                        ex = jnp.where(rel >= DH * v, kf[16 * v:16 * v + 16], ex)
                    p1 = [kd[0:16]] + [jnp.where(rel >= DH * v, kd[16 * v:16 * v + 16], kf[16 * v:16 * v + 16]) for v in range(1, 4)]
                    kw = jnp.concatenate([ex] + p1 + [k_scr[blk - 1, h]], axis=0)
                elif nt == 2:
                    kw = jnp.concatenate([kd, k_scr[blk - 1, h]], axis=0)
                else:
                    kw = kd
                kw = pltpu.bitcast(kw, bf16)
                st = lax.dot_general(kw, qw, NT, preferred_element_type=f32)
                mx = None
                for r in range(16):
                    if nt == 3:
                        v, r0 = r // 4, 8 * (r % 4)
                        msk = (lane8 >= 32 * v) & (lane8 < 32 * v + 32) & (sub8 + 8 * r > lane8)
                        s1 = jnp.where(msk, st[r0:r0 + 8], st[32 + 8 * r:32 + 8 * r + 8])
                    else:
                        s1 = jnp.where(sub8 + 8 * r <= lane8, st[8 * r:8 * r + 8], NEG)
                    s_scr[b, 8 * r:8 * r + 8, 128 * n:128 * (n + 1)] = s1
                    mx = s1 if mx is None else jnp.maximum(mx, s1)
                if nt >= 2:
                    base = 160 if nt == 3 else 128
                    for r in range(16):
                        s2 = st[base + 8 * r:base + 8 * r + 8]
                        s_scr[b, 128 + 8 * r:128 + 8 * r + 8, 128 * n:128 * (n + 1)] = s2
                        mx = jnp.maximum(mx, s2)
                ms.append(jnp.max(mx, axis=0, keepdims=True))
            st8[("m", u)] = jnp.concatenate(ms, axis=1)

        def softmax(u):
            sb, j = u
            nt = ntile(sb)
            b = (sb * NG + j) % (LOOK + 1)
            m = st8[("m", u)]
            acc = None
            far, mid, dia = [], [], []
            for c in range(8):
                p = jnp.exp2(s_scr[b, 16 * c:16 * c + 16, :] - m)
                if PMODE == "pack":
                    w = _pack(p[0:8], p[8:16])
                    if nt == 3:
                        wd = w & jnp.concatenate([m_scr[8 * c:8 * c + 8, :]] * 4, axis=1)
                        dia.append(wd)
                        far.append(w ^ wd)
                    else:
                        dia.append(w)
                else:
                    if nt == 3:
                        tri4 = jnp.concatenate([(sub16 + 16 * c) <= lane16] * 4, axis=1)
                        dia.append(jnp.where(tri4, p, 0.0))
                        far.append(jnp.where(tri4, 0.0, p))
                    else:
                        dia.append(p)
                if not ONES:
                    ps = p[0:8] + p[8:16]
                    acc = ps if acc is None else acc + ps
            if nt >= 2:
                for c in range(8):
                    p = jnp.exp2(s_scr[b, 128 + 16 * c:128 + 16 * c + 16, :] - m)
                    mid.append(_pack(p[0:8], p[8:16]) if PMODE == "pack" else p)
                    if not ONES:
                        acc = acc + (p[0:8] + p[8:16])
            st8[("p", u)] = jnp.concatenate(far + mid + dia, axis=0)
            if not ONES:
                st8[("il", u)] = pl.reciprocal(jnp.sum(acc, axis=0, keepdims=True), approx=True)

        def pv(u):
            sb, j = u
            nt = ntile(sb)
            tq = t0 + 128 * sb
            il = None if ONES else st8[("il", u)]
            pw = st8[("p", u)]
            on = []
            for n in range(4):
                rb = ((4 * j + n) * DH // 16) * 16
                cols = pl.ds(tq - 128 * (nt - 1), 128 * nt)
                vw = vt_scr[4 * j + n, :, cols] if ONES else vt_scr[rb:rb + 32, cols]
                if PMODE == "pack":
                    ph = pltpu.bitcast(pw[:, 128 * n:128 * (n + 1)], bf16)
                else:
                    ph = pw[:, 128 * n:128 * (n + 1)].astype(bf16)
                oh = _mm(vw, ph)
                if ONES:
                    lr = 0 if (4 * j + n) * DH - rb >= 4 else 24
                    on.append((rb, oh * pl.reciprocal(oh[lr:lr + 1], approx=True)))
                else:
                    on.append((rb, oh * il[:, 128 * n:128 * (n + 1)]))
            rows = []
            for r in range(10):
                r0 = 80 * j + 8 * r
                ha, hb = (8 * r) // DH, (8 * r + 7) // DH
                rba, oa = on[ha]
                va = oa[r0 - rba:r0 - rba + 8]
                if ha != hb:
                    rbb, ob = on[hb]
                    va = jnp.where(sub8 < (hb * DH - 8 * r), va, ob[r0 - rbb:r0 - rbb + 8])
                rows.append(va)
            ot_scr[80 * j:80 * j + 80, 128 * sb:128 * (sb + 1)] = jnp.concatenate(rows, axis=0)

        def gate():
            st8["g"] = jax.nn.sigmoid(jnp.sum(xs().astype(f32) * gw_ref[...].astype(f32).reshape(1, D), axis=-1, keepdims=True))

        def up(c):
            hh2 = 0.5 * _mm(xs(), w1_v[:, 128 * c:128 * (c + 1)])
            h_scr[:, 128 * c:128 * (c + 1)] = (hh2 * jnp.tanh(hh2) + hh2).astype(bf16)

        def down(n):
            b_scr[:, 128 * n:128 * (n + 1)] = (1.0 - st8["g"]) * _mm(h_scr[...], w2_v[:, 128 * n:128 * (n + 1)])

        def outproj(sb):
            r = slice(128 * sb, 128 * (sb + 1))
            o = ot_scr[:, r].T.astype(bf16)
            a = _mm(o, wo_v[...])
            o_v[pl.ds(t0 + 128 * sb, 128), :] = (st8["g"][r] * a + b_scr[r, :]).astype(bf16)
            o_copy(i * NSUB + sb).start()

        units = [(sb, j) for sb in range(NSUB) for j in range(NG)]
        nu = len(units)
        wait = lambda *cps: (lambda: [c.wait() for c in cps])
        if first:
            prog = [wait(cp_wk), kproj, wait(cp_wq), qproj] + [(k4, j) for j in range(4)] + [wait(cp_wv), vproj] + [(k4, j) for j in range(4, 8)] + [gate]
            fill = {k: [] for k in range(nu)}
        else:
            prog = [kproj, qproj, vproj] + [(k4, j) for j in range(8)] + [gate]
            fill = {k: [] for k in range(nu)}
            for c in range(12):
                fill[(c * (nu // 2)) // 12].append((up, c))
            dpos = [nu // 2 + (n * (nu // 2)) // 5 for n in range(5)]
            for n in range(5):
                fill[min(dpos[n] + (nu // 2) // 5, nu - 1)].append((down, n))
        prog += [(qk, units[k]) for k in range(LOOK)]
        for k in range(nu):
            if k + LOOK < nu:
                prog.append((qk, units[k + LOOK]))
            prog.append((softmax, units[k]))
            prog += fill[k]
            prog.append((pv, units[k]))
        if first:
            prog += [wait(*cp_w1)] + [(up, c) for c in range(12)] + [wait(cp_w2, cp_wo)] + [(down, n) for n in range(5)]
        prog += [(outproj, sb) for sb in range(NSUB)]
        for p in prog:
            if isinstance(p, tuple):
                p[0](p[1])
            else:
                p()

    x_copy(0).wait()
    step(0, True)
    def body(i, _):
        x_copy(i).wait()
        step(i, False)
        return _
    lax.fori_loop(1, NSTEP, body, 0)
    for i in range(S // 128):
        o_copy(i).wait()


@jax.jit
def pallas_gated_mix__sliding_block__dense_activation_silu__prompt_kernel(A_x, A_wqkv, A_wo, B_x, B_w1, B_w2, gate_w):
    x = A_x.reshape(S, D)
    gw = gate_w.reshape(1, D) if GW2D else gate_w
    anyspec = pl.BlockSpec(memory_space=pl.ANY)
    out = pl.pallas_call(
        kernel,
        in_specs=[anyspec, anyspec, anyspec, anyspec, anyspec, pl.BlockSpec(memory_space=pltpu.VMEM)],
        out_specs=anyspec,
        out_shape=jax.ShapeDtypeStruct((S, D), bf16),
        scratch_shapes=[
            pltpu.VMEM((S, D), bf16),
            pltpu.VMEM((D, D), bf16),
            pltpu.VMEM((D, D), bf16),
            pltpu.VMEM((D, D), bf16),
            pltpu.VMEM((D, D), bf16),
            pltpu.VMEM((D, F), bf16),
            pltpu.VMEM((F, D), bf16),
            pltpu.VMEM((S, D), bf16),
            pltpu.SemaphoreType.DMA((NSEM,)),
            pltpu.VMEM((S // 128, H, 64, 128), i32),
            pltpu.VMEM((H, 32, S) if ONES else (D, S), bf16),
            pltpu.VMEM((NG, TQ // 2, 128), i32),
            pltpu.VMEM((NG, TQ // 2, 128), i32),
            pltpu.VMEM((LOOK + 1, 256, 512), f32),
            pltpu.VMEM((TQ, F), bf16),
            pltpu.VMEM((TQ, D), f32),
            pltpu.VMEM((D, TQ), f32),
            pltpu.VMEM((64, 128), i32),
        ],
        compiler_params=pltpu.CompilerParams(vmem_limit_bytes=100 * 1024 * 1024, flags=FLAGS or None),
    )(x, A_wqkv, A_wo, B_w1, B_w2, gw)
    return out.reshape(1, S, D)
```

```python
import jax
import jax.numpy as jnp
from jax import lax
from jax.experimental import pallas as pl
from jax.experimental.pallas import tpu as pltpu

S, D, H, DH, F = 2048, 640, 32, 20, 1536
NSUB = 2
TQ = 128 * NSUB
NSTEP = S // TQ
NG = H // 4
LOOK = 2
QSCALE = DH ** -0.5 * 1.4426950408889634
NEG = -1e30
NT = (((1,), (1,)), ((), ()))
f32, bf16, i32 = jnp.float32, jnp.bfloat16, jnp.int32
OFFS = (0, 16, 32, 48, 0, 16, 32, 48)
SEM_X, SEM_W, SEM_OUT = 0, NSTEP, NSTEP + 6
NSEM = SEM_OUT + S // 128


def _mm(a, b):
    return jnp.dot(a, b, preferred_element_type=f32)


def _roll(a, shift):
    return a if shift == 0 else pltpu.roll(a, shift, 1)


def _words(a):
    return pltpu.bitcast(a.astype(bf16), i32)


def _regroup(a):
    lane = lax.broadcasted_iota(i32, (a.shape[0], 128), 1)
    t = [a[:, 128 * n:128 * (n + 1)] for n in range(5)]
    r = [pltpu.roll(x, 64, 1) for x in t]
    sh = [jnp.where(lane < 64, r[n], r[n + 1]) for n in range(4)]
    return [t[0], sh[0], t[1], sh[1], sh[2], t[3], sh[3], t[4]]


def _kernel(x_hbm, wqkv_hbm, wo_hbm, w1_hbm, w2_hbm, gw_ref, o_hbm,
            x_v, wq_v, wk_v, wv_v, wo_v, w1_v, w2_v, o_v, sems,
            k_scr, vt_scr, kraw_scr, q_scr, s_scr, h_scr, b_scr, ot_scr, v_scr):

    def x_copy(i):
        r = pl.ds(pl.multiple_of(i * TQ, TQ), TQ)
        return pltpu.make_async_copy(x_hbm.at[r, :], x_v.at[r, :], sems.at[SEM_X + i])

    def o_copy(i):
        r = pl.ds(pl.multiple_of(i * 128, 128), 128)
        return pltpu.make_async_copy(o_v.at[r, :], o_hbm.at[r, :], sems.at[SEM_OUT + i])

    cp_wk = pltpu.make_async_copy(wqkv_hbm.at[:, D:2 * D], wk_v, sems.at[SEM_W])
    cp_wq = pltpu.make_async_copy(wqkv_hbm.at[:, 0:D], wq_v, sems.at[SEM_W + 1])
    cp_wv = pltpu.make_async_copy(wqkv_hbm.at[:, 2 * D:3 * D], wv_v, sems.at[SEM_W + 2])
    cp_w1 = pltpu.make_async_copy(w1_hbm, w1_v, sems.at[SEM_W + 3])
    cp_w2 = pltpu.make_async_copy(w2_hbm, w2_v, sems.at[SEM_W + 4])
    cp_wo = pltpu.make_async_copy(wo_hbm, wo_v, sems.at[SEM_W + 5])
    x_copy(0).start()
    for cp in (cp_wk, cp_wq, cp_wv, cp_w1, cp_w2, cp_wo):
        cp.start()
    for i in range(1, NSTEP):
        x_copy(i).start()

    def step(i, first):
        t0 = i * TQ if first else pl.multiple_of(i * TQ, TQ)
        sub8 = lax.broadcasted_iota(i32, (8, 128), 0)
        lane8 = lax.broadcasted_iota(i32, (8, 128), 1)
        sub16 = lax.broadcasted_iota(i32, (16, 128), 0)
        lane16 = lax.broadcasted_iota(i32, (16, 128), 1)
        val = {}
        units = [(sb, j) for sb in range(NSUB) for j in range(NG)]

        def xs():
            return x_v[pl.ds(t0, TQ), :]

        def ntile(sb):
            return min(3, sb + 1) if first else 3

        def kproj():
            for j, t in enumerate(_regroup(_mm(xs(), wk_v[...]))):
                kraw_scr[j] = _words(t)

        def qproj():
            for j, t in enumerate(_regroup(_mm(xs(), wq_v[...]) * QSCALE)):
                q_scr[j] = _words(t)

        def vproj():
            v_scr[...] = _mm(xs(), wv_v[...])
            vt = v_scr[...].T
            row = lax.broadcasted_iota(i32, (32, TQ), 0)
            for h in range(H):
                rb = h * DH // 16 * 16
                o = h * DH - rb
                vt_scr[h, :, pl.ds(t0, TQ)] = jnp.where((row >= o) & (row < o + DH), vt[rb:rb + 32], 1.0).astype(bf16)

        def krep(j):
            lane = lax.broadcasted_iota(i32, (TQ // 2, 128), 1)
            kw = kraw_scr[j]
            for n in range(4):
                a = jnp.where(((lane - (OFFS[j] + DH * n)) & 127) < DH, kw, 0)
                a = a | _roll(a, DH)
                a = a | _roll(a, 2 * DH)
                for sb in range(NSUB):
                    k_scr[i * NSUB + sb, 4 * j + n] = a[64 * sb:64 * (sb + 1)]

        def gate():
            gw = gw_ref[...].astype(f32).reshape(1, D)
            val["g"] = jax.nn.sigmoid(jnp.sum(xs().astype(f32) * gw, axis=-1, keepdims=True))

        def qk(u):
            sb, j = units[u]
            nt = ntile(sb)
            blk = i * NSUB + sb
            buf = u % (LOOK + 1)
            qv = q_scr[j, 64 * sb:64 * (sb + 1), :]
            ms = []
            for n in range(4):
                h = 4 * j + n
                rel = (lane16 - (OFFS[j] + DH * n)) & 127
                qw = jnp.concatenate(
                    [jnp.where((rel >= DH * v) & (rel < DH * (v + 1)), _roll(qv[16 * v:16 * v + 16], DH * v), 0)
                     for v in range(4)], axis=0)
                kd = k_scr[blk, h]
                if nt == 3:
                    kf = k_scr[blk - 2, h]
                    ex = kf[0:16]
                    for v in range(1, 4):
                        ex = jnp.where(rel >= DH * v, kf[16 * v:16 * v + 16], ex)
                    mg = [kd[0:16]] + [jnp.where(rel >= DH * v, kd[16 * v:16 * v + 16], kf[16 * v:16 * v + 16])
                                       for v in range(1, 4)]
                    kw = jnp.concatenate([ex] + mg + [k_scr[blk - 1, h]], axis=0)
                elif nt == 2:
                    kw = jnp.concatenate([kd, k_scr[blk - 1, h]], axis=0)
                else:
                    kw = kd
                st = lax.dot_general(pltpu.bitcast(kw, bf16), pltpu.bitcast(qw, bf16), NT,
                                     preferred_element_type=f32)
                mx = None
                for r in range(16):
                    if nt == 3:
                        v, r0 = r // 4, 8 * (r % 4)
                        far = (lane8 >= 32 * v) & (lane8 < 32 * v + 32) & (sub8 + 8 * r > lane8)
                        s1 = jnp.where(far, st[r0:r0 + 8], st[32 + 8 * r:32 + 8 * r + 8])
                    else:
                        s1 = jnp.where(sub8 + 8 * r <= lane8, st[8 * r:8 * r + 8], NEG)
                    s_scr[buf, 8 * r:8 * r + 8, 128 * n:128 * (n + 1)] = s1
                    mx = s1 if mx is None else jnp.maximum(mx, s1)
                if nt >= 2:
                    base = 160 if nt == 3 else 128
                    for r in range(16):
                        s2 = st[base + 8 * r:base + 8 * r + 8]
                        s_scr[buf, 128 + 8 * r:128 + 8 * r + 8, 128 * n:128 * (n + 1)] = s2
                        mx = jnp.maximum(mx, s2)
                ms.append(jnp.max(mx, axis=0, keepdims=True))
            val["m", u] = jnp.concatenate(ms, axis=1)

        def softmax(u):
            sb, _ = units[u]
            nt = ntile(sb)
            buf = u % (LOOK + 1)
            m = val["m", u]
            far, mid, dia = [], [], []
            for c in range(8):
                p = jnp.exp2(s_scr[buf, 16 * c:16 * c + 16, :] - m)
                if nt == 3:
                    tri = jnp.concatenate([(sub16 + 16 * c) <= lane16] * 4, axis=1)
                    dia.append(jnp.where(tri, p, 0.0))
                    far.append(jnp.where(tri, 0.0, p))
                else:
                    dia.append(p)
            if nt >= 2:
                for c in range(8):
                    mid.append(jnp.exp2(s_scr[buf, 128 + 16 * c:128 + 16 * c + 16, :] - m))
            val["p", u] = jnp.concatenate(far + mid + dia, axis=0)

        def pv(u):
            sb, j = units[u]
            nt = ntile(sb)
            cols = pl.ds(t0 + 128 * sb - 128 * (nt - 1), 128 * nt)
            pw = val["p", u]
            on = []
            for n in range(4):
                h = 4 * j + n
                rb = h * DH // 16 * 16
                oh = _mm(vt_scr[h, :, cols], pw[:, 128 * n:128 * (n + 1)].astype(bf16))
                lr = 0 if h * DH - rb >= 4 else 24
                on.append((rb, oh * (1.0 / oh[lr:lr + 1])))
            rows = []
            for r in range(10):
                r0 = 80 * j + 8 * r
                ha, hb = 8 * r // DH, (8 * r + 7) // DH
                rba, oa = on[ha]
                va = oa[r0 - rba:r0 - rba + 8]
                if ha != hb:
                    rbb, ob = on[hb]
                    va = jnp.where(sub8 < hb * DH - 8 * r, va, ob[r0 - rbb:r0 - rbb + 8])
                rows.append(va)
            ot_scr[80 * j:80 * j + 80, 128 * sb:128 * (sb + 1)] = jnp.concatenate(rows, axis=0)

        def up(c):
            hh = 0.5 * _mm(xs(), w1_v[:, 128 * c:128 * (c + 1)])
            h_scr[:, 128 * c:128 * (c + 1)] = (hh * jnp.tanh(hh) + hh).astype(bf16)

        def down(n):
            b_scr[:, 128 * n:128 * (n + 1)] = (1.0 - val["g"]) * _mm(h_scr[...], w2_v[:, 128 * n:128 * (n + 1)])

        def outproj(sb):
            r = slice(128 * sb, 128 * (sb + 1))
            a = _mm(ot_scr[:, r].T.astype(bf16), wo_v[...])
            o_v[pl.ds(t0 + 128 * sb, 128), :] = (val["g"][r] * a + b_scr[r, :]).astype(bf16)
            o_copy(i * NSUB + sb).start()

        nu = len(units)
        if first:
            cp_wk.wait(); kproj()
            cp_wq.wait(); qproj(); krep(0); krep(1)
            cp_wv.wait(); vproj(); krep(2); gate()
            for u in range(LOOK):
                qk(u)
            for u in range(nu):
                if u + LOOK < nu:
                    if 3 <= u + LOOK < NG:
                        krep(u + LOOK)
                    qk(u + LOOK)
                softmax(u)
                pv(u)
            cp_w1.wait()
            for c in range(F // 128):
                up(c)
            cp_w2.wait(); cp_wo.wait()
            for n in range(D // 128):
                down(n)
        else:
            kproj(); qproj(); vproj()
            for j in range(NG):
                krep(j)
            gate()
            up_at = (0, 0, 1, 2, 2, 3, 4, 4, 5, 6, 6, 7)
            down_at = (9, 10, 12, 13, 15)
            for u in range(LOOK):
                qk(u)
            for u in range(nu):
                if u + LOOK < nu:
                    qk(u + LOOK)
                softmax(u)
                for c in range(F // 128):
                    if up_at[c] == u:
                        up(c)
                for n in range(D // 128):
                    if down_at[n] == u:
                        down(n)
                pv(u)
        for sb in range(NSUB):
            outproj(sb)

    x_copy(0).wait()
    step(0, True)

    def body(i, carry):
        x_copy(i).wait()
        step(i, False)
        return carry

    lax.fori_loop(1, NSTEP, body, 0)
    for i in range(S // 128):
        o_copy(i).wait()


@jax.jit
def pallas_gated_mix__sliding_block__dense_activation_silu__prompt_kernel(
    A_x: jax.Array,
    A_wqkv: jax.Array,
    A_wo: jax.Array,
    B_x: jax.Array,
    B_w1: jax.Array,
    B_w2: jax.Array,
    gate_w: jax.Array,
):
    del B_x
    hbm = pl.BlockSpec(memory_space=pl.ANY)
    out = pl.pallas_call(
        _kernel,
        in_specs=[hbm, hbm, hbm, hbm, hbm, pl.BlockSpec(memory_space=pltpu.VMEM)],
        out_specs=hbm,
        out_shape=jax.ShapeDtypeStruct((S, D), bf16),
        scratch_shapes=[
            pltpu.VMEM((S, D), bf16),
            pltpu.VMEM((D, D), bf16),
            pltpu.VMEM((D, D), bf16),
            pltpu.VMEM((D, D), bf16),
            pltpu.VMEM((D, D), bf16),
            pltpu.VMEM((D, F), bf16),
            pltpu.VMEM((F, D), bf16),
            pltpu.VMEM((S, D), bf16),
            pltpu.SemaphoreType.DMA((NSEM,)),
            pltpu.VMEM((S // 128, H, 64, 128), i32),
            pltpu.VMEM((H, 32, S), bf16),
            pltpu.VMEM((NG, TQ // 2, 128), i32),
            pltpu.VMEM((NG, TQ // 2, 128), i32),
            pltpu.VMEM((LOOK + 1, 256, 512), f32),
            pltpu.VMEM((TQ, F), bf16),
            pltpu.VMEM((TQ, D), f32),
            pltpu.VMEM((D, TQ), f32),
            pltpu.VMEM((TQ, D), f32),
        ],
        compiler_params=pltpu.CompilerParams(vmem_limit_bytes=64 * 1024 * 1024),
    )(A_x.reshape(S, D), A_wqkv, A_wo, B_w1, B_w2, gate_w)
    return out.reshape(1, S, D)
```
